```python
import jax
import jax.numpy as jnp

def _softmax(x, axis=-1):
    return jax.nn.softmax(x, axis=axis)
def _gelu(x):
    return jax.nn.gelu(x, approximate=True)
def _silu(x):
    return jax.nn.silu(x)
def _sigmoid(x):
    return jax.nn.sigmoid(x)
def _layernorm(x, axis=-1, eps=1e-5):
    m = jnp.mean(x, axis=axis, keepdims=True)
    v = jnp.var(x, axis=axis, keepdims=True)
    return (x - m) / jnp.sqrt(v + eps)
def _scatter_add(tgt, idx, src, axis=0):
    return tgt.at[idx].add(src)
def _segment_sum(src, seg, n):
    return jax.ops.segment_sum(src, seg, n)
class _Rng:
    def __init__(self, key):
        self._k = key
    def _next(self):
        self._k, sub = jax.random.split(self._k)
        return sub
    def normal(self, shape):
        return jax.random.normal(self._next(), shape, dtype=jnp.bfloat16)
    def randint(self, lo, hi, shape):
        return jax.random.randint(self._next(), shape, lo, hi, dtype=jnp.int32)
    def uniform(self, shape, lo=0.0, hi=1.0):
        return jax.random.uniform(self._next(), shape, jnp.bfloat16, lo, hi)
    def permutation(self, n):
        return jax.random.permutation(self._next(), n)


kernel_name = 'standalone__detection_seg_fpn_lateral__vision'

def setup_inputs():
    _rng = _Rng(jax.random.key(int.from_bytes(__import__("os").urandom(4), "little")))
    _w = (lambda a: (lambda t: t.astype(jnp.bfloat16) if jnp.issubdtype(t.dtype, jnp.floating) else t)(jnp.asarray(a)))
    H = W = (384 // 2) * 2
    C = 384
    k = 1
    return {
        "c_fine": _w((lambda *s: _rng.normal(s) * 0.05)(1, H, W, C)),
        "p_coarse": _w((lambda *s: _rng.normal(s) * 0.05)(1, H // 2, W // 2, C)),
        "w_lat": _w((lambda *s: _rng.normal(s) * 0.05)(C, C)),
        "w_out": _w((lambda *s: _rng.normal(s) * 0.05)(k, k, C, C)),
    }

def reference(c_fine, p_coarse, w_lat, w_out):
    B, H, W, C = c_fine.shape
    k = 1
    lat = jnp.einsum("bhwc,cd->bhwd", c_fine, w_lat)
    up = jnp.repeat(jnp.repeat(p_coarse, 2, axis=1), 2, axis=2)
    m = lat + up
    pad = k // 2
    mp = jnp.pad(m, ((0, 0), (pad, pad), (pad, pad), (0, 0)))
    o = None
    for di in range(k):
        for dj in range(k):
            t = jnp.einsum("bhwc,cd->bhwd", mp[:, di:di + H, dj:dj + W, :], w_out[di, dj])
            o = t if o is None else o + t
    return o
```

```python
import jax
import jax.numpy as jnp
from jax import lax
import jax.experimental.pallas as pl
import jax.experimental.pallas.tpu as pltpu

_BLOCK = 32
_STEP = 2
_PIECE = 4
_RUN = 48
_W_AT, _R_AT, _DRIFT = 4.0, 20.0, 3.1
_R1_AT = 8


@jax.jit
def pallas_standalone__detection_seg_fpn_lateral__vision_kernel(
    c_fine: jax.Array,
    p_coarse: jax.Array,
    w_lat: jax.Array,
    w_out: jax.Array,
):
    B, H, W, C = c_fine.shape
    Wc = W // 2
    units = B * H // 2
    D = w_out.shape[-1]
    dt = c_fine.dtype
    f32 = jnp.float32

    n_blocks = units // _BLOCK
    steps = _BLOCK // _STEP
    pieces = _BLOCK // _PIECE
    piece_steps = _PIECE // _STEP
    strips = 2 * W // _RUN
    assert n_blocks * _BLOCK == units and n_blocks >= 2 and strips * _RUN == 2 * W
    w_step = [int((_W_AT + _DRIFT * s) // _STEP) for s in range(n_blocks - 1)]
    r_step = [int((_R_AT + _DRIFT * s) // _STEP) for s in range(n_blocks - 2)]
    assert all(w < r < steps for w, r in zip(w_step, r_step)) and w_step[-1] < steps

    def lookup(table, s):
        v = jnp.int32(steps)
        for t, entry in enumerate(table):
            v = jnp.where(s == t + 1, jnp.int32(entry), v)
        return v

    def kernel(c_hbm, p_hbm, wl_hbm, wo_hbm, o_hbm,
               c_buf, p_buf, o_buf, wl_buf, wo_buf, wf_buf,
               c_sem, p_sem, o_sem, w_sem):

        def read_copies(s, k):
            slot = s % 2
            src = pl.ds(s * _BLOCK + k * _PIECE, _PIECE)
            dst = pl.ds(k * _PIECE, _PIECE)
            return (
                pltpu.make_async_copy(p_hbm.at[src], p_buf.at[slot, dst], p_sem.at[slot, k]),
                pltpu.make_async_copy(c_hbm.at[src], c_buf.at[slot, dst], c_sem.at[slot, k]),
            )

        def write_copy(s, q):
            slot = s % 2
            cols = pl.ds(q * _RUN, _RUN)
            return pltpu.make_async_copy(
                o_buf.at[slot, :, cols],
                o_hbm.at[pl.ds(s * _BLOCK, _BLOCK), cols],
                o_sem.at[slot, q],
            )

        def read_start(s):
            for k in range(pieces):
                for cp in read_copies(s, k):
                    cp.start(priority=1)

        def read_wait(s, k):
            for cp in read_copies(s, k):
                cp.wait()

        def write_start(s):
            for q in range(strips):
                write_copy(s, q).start(priority=1)

        def write_wait(s):
            for q in range(strips):
                write_copy(s, q).wait()

        weights = (
            pltpu.make_async_copy(wl_hbm, wl_buf, w_sem.at[0]),
            pltpu.make_async_copy(wo_hbm, wo_buf, w_sem.at[1]),
        )
        for cp in weights:
            cp.start()
        read_start(0)
        for cp in weights:
            cp.wait()
        wf_buf[...] = jnp.dot(
            wl_buf[...], wo_buf[...], preferred_element_type=f32
        ).astype(dt)

        def step(i, carry):
            s = i // steps
            j = i % steps
            slot = s % 2
            j_write = lookup(w_step, s)
            j_read = lookup(r_step, s)

            @pl.when(i == _R1_AT // _STEP)
            def _():
                read_start(1)

            @pl.when(j == j_write)
            def _():
                for k in range(pieces):
                    @pl.when(k * piece_steps >= j)
                    def _():
                        read_wait(s, k)
                write_start(s - 1)

            @pl.when(j == j_read)
            def _():
                write_wait(s - 1)
                read_start(s + 1)

            @pl.when((j % piece_steps == 0) & (j < j_write))
            def _():
                read_wait(s, j // piece_steps)

            for r in range(_STEP):
                u = j * _STEP + r
                q = jnp.dot(p_buf[slot, u], wo_buf[...], preferred_element_type=f32)
                for rows in (pl.ds(0, W), pl.ds(W, W)):
                    x = pltpu.bitcast(c_buf[slot, u, rows, :], jnp.uint32)
                    halves = [
                        pltpu.unpack_elementwise(
                            x, index=h, packed_dtype=dt, unpacked_dtype=f32)
                        for h in range(2)
                    ]
                    y = jnp.dot(
                        jnp.concatenate(halves, axis=0).astype(dt),
                        wf_buf[...], preferred_element_type=f32)
                    o = pltpu.pack_elementwise(
                        [y[:Wc] + q, y[Wc:] + q], packed_dtype=dt)
                    o_buf[slot, u, rows, :] = pltpu.bitcast(o, dt)
            return carry

        lax.fori_loop(0, n_blocks * steps, step, 0)
        write_start(n_blocks - 1)
        write_wait(n_blocks - 2)
        write_wait(n_blocks - 1)

    out = pl.pallas_call(
        kernel,
        in_specs=[pl.BlockSpec(memory_space=pl.ANY)] * 4,
        out_specs=pl.BlockSpec(memory_space=pl.ANY),
        out_shape=jax.ShapeDtypeStruct((units, 2 * W, D), dt),
        scratch_shapes=[
            pltpu.VMEM((2, _BLOCK, 2 * W, C), dt),
            pltpu.VMEM((2, _BLOCK, Wc, w_lat.shape[1]), dt),
            pltpu.VMEM((2, _BLOCK, 2 * W, D), dt),
            pltpu.VMEM(w_lat.shape, dt),
            pltpu.VMEM(w_out.shape[2:], dt),
            pltpu.VMEM((C, D), dt),
            pltpu.SemaphoreType.DMA((2, pieces)),
            pltpu.SemaphoreType.DMA((2, pieces)),
            pltpu.SemaphoreType.DMA((2, strips)),
            pltpu.SemaphoreType.DMA((2,)),
        ],
        compiler_params=pltpu.CompilerParams(vmem_limit_bytes=100 * 1024 * 1024),
    )(
        c_fine.reshape(units, 2 * W, C),
        p_coarse.reshape(units, Wc, p_coarse.shape[-1]),
        w_lat,
        w_out.reshape(w_out.shape[2:]),
    )
    return out.reshape(B, H, W, D)
```

```python
import jax
import jax.numpy as jnp
from jax import lax
import jax.experimental.pallas as pl
import jax.experimental.pallas.tpu as pltpu

_STEP = 2
_PIECE = 4
_GROUP = 8
_IN_SLOTS = 16
_OUT_SLOTS = 12
_RUN = 48
_DOTS = 3
_PARTS = 4
_FETCHES = 12
_TAIL = 640
_AHEAD = 3
_READ1_PIECES, _WRITE1_GROUPS = 32, 10
_WRITE1_AT, _READ2_AT, _WRITE2_AT = 37, 57, 76


def _rem(a, n):
    return a % n if isinstance(a, int) else lax.rem(a, n)


def _slot_free_at(piece):
    return 2 * (piece - _IN_SLOTS + 1)


def _plan(steps, pieces, groups):
    per_step = _PARTS * _STEP
    split = 2 * _READ1_PIECES
    bulk1 = pl.cdiv(split * per_step - _WRITE1_AT * _FETCHES, per_step)
    bulk2 = pl.cdiv(
        (steps - split) * per_step - (_WRITE2_AT - _READ2_AT) * _FETCHES, per_step)
    assert bulk1 >= 1 and bulk2 >= 1
    for start, first, last, end in ((0, bulk1, split, _WRITE1_AT),
                                    (_READ2_AT, split + bulk2, steps, _WRITE2_AT)):
        assert _slot_free_at((first - 1) // 2) <= start
        for n in range(first * per_step, last * per_step):
            at = start + (n - first * per_step) // _FETCHES
            assert _slot_free_at(n // (2 * per_step)) <= at < min(end, n // per_step)
    assert _IN_SLOTS < _READ1_PIECES < pieces
    assert _slot_free_at(_READ1_PIECES - 1) < _WRITE1_AT < _READ2_AT < split
    assert _READ2_AT < _slot_free_at(pieces - 1) < _WRITE2_AT <= steps - 2

    written_at = {g: _WRITE1_AT for g in range(_AHEAD)}
    written_at.update({_WRITE1_GROUPS + g: _WRITE2_AT for g in range(_AHEAD)})
    for i in range(0, steps, 2):
        if i > _WRITE2_AT:
            written_at[_WRITE1_GROUPS + _AHEAD - 1 + i // 2 - _WRITE2_AT // 2] = i
        elif i > _WRITE1_AT and _AHEAD - 1 + i // 2 - _WRITE1_AT // 2 < _WRITE1_GROUPS:
            written_at[_AHEAD - 1 + i // 2 - _WRITE1_AT // 2] = i
    in_loop = len(written_at)
    assert sorted(written_at) == list(range(in_loop))
    assert groups - _OUT_SLOTS <= in_loop < groups
    assert all(4 * (g + 1) <= at < 4 * (g + _OUT_SLOTS) for g, at in written_at.items())
    assert written_at[_WRITE1_GROUPS - 1] < _READ2_AT
    assert _READ2_AT < 4 * (_WRITE1_GROUPS - 1 + _OUT_SLOTS) < steps
    return bulk1, bulk2, in_loop


@jax.jit
def pallas_standalone__detection_seg_fpn_lateral__vision_kernel(
    c_fine: jax.Array,
    p_coarse: jax.Array,
    w_lat: jax.Array,
    w_out: jax.Array,
):
    B, H, W, C = c_fine.shape
    Wc = W // 2
    units = B * H // 2
    bf16, f32 = jnp.bfloat16, jnp.float32
    assert c_fine.dtype == bf16 and units % _GROUP == 0

    steps, pieces, groups = units // _STEP, units // _PIECE, units // _GROUP
    bulk1, bulk2, groups_in_loop = _plan(steps, pieces, groups)
    last_pieces = (_READ1_PIECES - 1, pieces - 1)
    split = 2 * _READ1_PIECES
    per_step = _PARTS * _STEP
    part_rows = Wc // _PARTS
    dot_rows = 2 * W // _DOTS
    fine, coarse = pl.ds(0, 2 * W), pl.ds(2 * W, Wc)

    def kernel(c_hbm, p_hbm, wl_hbm, wo_hbm, o_hbm,
               in_buf, out_buf, wl_buf, wo_buf, wf_buf,
               c_sem, head_sem, p_sem, o_sem, w_sem):

        def piece_copy(k):
            slot = _rem(k, _IN_SLOTS)
            return pltpu.make_async_copy(
                c_hbm.at[pl.ds(k * _PIECE, _PIECE)],
                in_buf.at[pl.ds(slot * _PIECE, _PIECE), fine],
                c_sem.at[slot])

        def head_copies(k):
            u, slot = k * _PIECE, _rem(k, _IN_SLOTS) * _PIECE
            head = pl.ds(0, 2 * W - _TAIL)
            return (
                pltpu.make_async_copy(
                    c_hbm.at[pl.ds(u, _PIECE - 1)],
                    in_buf.at[pl.ds(slot, _PIECE - 1), fine], head_sem),
                pltpu.make_async_copy(
                    c_hbm.at[u + _PIECE - 1, head],
                    in_buf.at[slot + _PIECE - 1, head], head_sem),
            )

        def tail_copy(k):
            slot = _rem(k, _IN_SLOTS)
            tail = pl.ds(2 * W - _TAIL, _TAIL)
            return pltpu.make_async_copy(
                c_hbm.at[k * _PIECE + _PIECE - 1, tail],
                in_buf.at[slot * _PIECE + _PIECE - 1, tail], c_sem.at[slot])

        def coarse_step_copy(i):
            slot = _rem(i, 2 * _IN_SLOTS)
            return pltpu.make_async_copy(
                p_hbm.at[pl.ds(i * _STEP, _STEP)],
                in_buf.at[pl.ds(slot * _STEP, _STEP), coarse],
                p_sem.at[slot])

        def coarse_part_copy(n):
            u = lax.div(n, _PARTS)
            slot = lax.rem(u, _IN_SLOTS * _PIECE)
            row = pl.multiple_of(lax.rem(n, _PARTS) * part_rows, part_rows)
            return pltpu.make_async_copy(
                p_hbm.at[u, pl.ds(row, part_rows)],
                in_buf.at[slot, pl.ds(2 * W + row, part_rows)],
                p_sem.at[lax.div(slot, _STEP)])

        def write_start(g):
            slot = _rem(g, _OUT_SLOTS)
            for start in range(0, 2 * W, _RUN):
                cols = pl.ds(start, _RUN)
                pltpu.make_async_copy(
                    out_buf.at[pl.ds(slot * _GROUP, _GROUP), cols],
                    o_hbm.at[pl.ds(g * _GROUP, _GROUP), cols],
                    o_sem.at[slot]).start(priority=1)

        def write_wait(g):
            slot = _rem(g, _OUT_SLOTS)
            buf = out_buf.at[pl.ds(slot * _GROUP, _GROUP)]
            pltpu.make_async_copy(buf, buf, o_sem.at[slot]).wait()

        weights = (
            pltpu.make_async_copy(wl_hbm, wl_buf, w_sem.at[0]),
            pltpu.make_async_copy(wo_hbm, wo_buf, w_sem.at[1]),
        )
        for copy in weights:
            copy.start()
        piece_copy(0).start(priority=1)

        @pl.loop(0, bulk1)
        def _(i):
            coarse_step_copy(i).start(priority=1)

        @pl.loop(1, _IN_SLOTS)
        def _(k):
            piece_copy(k).start(priority=1)

        for copy in weights:
            copy.wait()
        wf_buf[...] = jnp.dot(
            wl_buf[...], wo_buf[...], preferred_element_type=f32).astype(bf16)

        @pl.loop(0, steps)
        def _(i):
            @pl.when((i == _WRITE1_AT) | (i == _WRITE2_AT))
            def _():
                first = i == _WRITE1_AT
                for copy in head_copies(jnp.where(first, *last_pieces)):
                    copy.wait()
                g0 = jnp.where(first, 0, _WRITE1_GROUPS)

                @pl.loop(0, _AHEAD)
                def _(n):
                    write_start(g0 + n)

            @pl.when(i == _READ2_AT)
            def _():
                write_wait(_WRITE1_GROUPS - 1)

                @pl.loop(split, split + bulk2)
                def _(n):
                    coarse_step_copy(n).start(priority=1)

                @pl.loop(_READ1_PIECES, _READ2_AT // 2 + _IN_SLOTS)
                def _(k):
                    piece_copy(k).start(priority=1)

            @pl.when((i & 1) == 0)
            def _():
                k = i >> 1
                nxt = k + (_IN_SLOTS - 1)

                @pl.when(((i > 0) & (nxt < last_pieces[0]))
                         | ((i > _READ2_AT) & (nxt < last_pieces[1])))
                def _():
                    piece_copy(nxt).start(priority=1)

                for last in last_pieces:
                    @pl.when(nxt == last)
                    def _():
                        for copy in head_copies(last):
                            copy.start(priority=1)
                        tail_copy(last).start(priority=1)

                g = k + jnp.where(
                    i > _WRITE2_AT,
                    _WRITE1_GROUPS + _AHEAD - 1 - _WRITE2_AT // 2,
                    _AHEAD - 1 - _WRITE1_AT // 2)

                @pl.when((i > _WRITE2_AT) | ((i > _WRITE1_AT) & (g < _WRITE1_GROUPS)))
                def _():
                    write_start(g)

                @pl.when((k != last_pieces[0]) & (k != last_pieces[1]))
                def _():
                    piece_copy(k).wait()

                for last in last_pieces:
                    @pl.when(k == last)
                    def _():
                        tail_copy(last).wait()

                old = (i >> 2) - _OUT_SLOTS

                @pl.when(((i & 3) == 0) & (old >= 0) & (old != _WRITE1_GROUPS - 1))
                def _():
                    write_wait(old)

            coarse_step_copy(i).wait()

            second = i >= _READ2_AT
            n0 = i * _FETCHES + jnp.where(
                second,
                (split + bulk2) * per_step - _READ2_AT * _FETCHES,
                bulk1 * per_step)
            n_end = jnp.where(second, steps * per_step, split * per_step)
            fetched = []

            def load(u, start, size):
                n = n0 + len(fetched)
                fetched.append(n)

                @pl.when(n < n_end)
                def _():
                    coarse_part_copy(n).start()

                return in_buf[u, pl.ds(start, size), :]

            u_in = lax.rem(i, 2 * _IN_SLOTS) * _STEP
            u_out = lax.rem(i, 4 * _OUT_SLOTS) * _STEP
            half = dot_rows // 2
            for r in range(_STEP):
                q = jnp.dot(load(u_in + r, 2 * W, Wc), wo_buf[...],
                            preferred_element_type=f32)
                q = jnp.concatenate([q, q], axis=0)
                for t in range(_DOTS):
                    start = t * dot_rows
                    if t == 0:
                        x = load(u_in + r, start, dot_rows)
                    else:
                        x = jnp.concatenate(
                            [load(u_in + r, start, half),
                             load(u_in + r, start + half, half)], axis=0)
                    x = pltpu.bitcast(x, jnp.uint32)
                    even = lax.bitcast_convert_type(x << 16, f32)
                    odd = lax.bitcast_convert_type(x & jnp.uint32(0xFFFF0000), f32)
                    y = jnp.dot(
                        jnp.concatenate([even, odd], axis=0).astype(bf16),
                        wf_buf[...], preferred_element_type=f32)
                    up = q[t * half:(t + 1) * half]
                    even, odd = (
                        lax.bitcast_convert_type(
                            (v + up).astype(bf16).astype(f32), jnp.uint32)
                        for v in (y[:half], y[half:]))
                    out_buf[u_out + r, pl.ds(start, dot_rows), :] = pltpu.bitcast(
                        (even >> 16) | odd, bf16)
            assert len(fetched) == _FETCHES

        @pl.loop(groups_in_loop, groups)
        def _(g):
            write_start(g)

        @pl.loop(groups - _OUT_SLOTS, groups)
        def _(g):
            write_wait(g)

    out = pl.pallas_call(
        kernel,
        in_specs=[pl.BlockSpec(memory_space=pl.ANY)] * 4,
        out_specs=pl.BlockSpec(memory_space=pl.ANY),
        out_shape=jax.ShapeDtypeStruct((units, 2 * W, C), bf16),
        scratch_shapes=[
            pltpu.VMEM((_IN_SLOTS * _PIECE, 2 * W + Wc, C), bf16),
            pltpu.VMEM((_OUT_SLOTS * _GROUP, 2 * W, C), bf16),
            pltpu.VMEM((C, C), bf16),
            pltpu.VMEM((C, C), bf16),
            pltpu.VMEM((C, C), bf16),
            pltpu.SemaphoreType.DMA((_IN_SLOTS,)),
            pltpu.SemaphoreType.DMA(()),
            pltpu.SemaphoreType.DMA((2 * _IN_SLOTS,)),
            pltpu.SemaphoreType.DMA((_OUT_SLOTS,)),
            pltpu.SemaphoreType.DMA((2,)),
        ],
        compiler_params=pltpu.CompilerParams(
            vmem_limit_bytes=110 * 1024 * 1024, disable_bounds_checks=True),
    )(
        c_fine.reshape(units, 2 * W, C),
        p_coarse.reshape(units, Wc, C),
        w_lat,
        w_out.reshape(C, C),
    )
    return out.reshape(B, H, W, C)
```

```python
import jax
import jax.numpy as jnp
from jax import lax
import jax.experimental.pallas as pl
import jax.experimental.pallas.tpu as pltpu

_STEP = 2
_PIECE = 4
_GROUP = 8
_IN_SLOTS = 16
_OUT_SLOTS = 12
_RUN = 48
_DOTS = 3
_PARTS = 4
_FETCHES = 12
_TAIL = 640
_AHEAD = 3
_READ1_PIECES, _WRITE1_GROUPS = 32, 10
_WRITE1_AT, _READ2_AT, _WRITE2_AT = 37, 57, 76


def _rem(a, n):
    return a % n if isinstance(a, int) else lax.rem(a, n)


def _slot_free_at(piece):
    return 2 * (piece - _IN_SLOTS + 1)


def _plan(steps, pieces, groups):
    per_step = _PARTS * _STEP
    split = 2 * _READ1_PIECES
    bulk1 = pl.cdiv(split * per_step - _WRITE1_AT * _FETCHES, per_step)
    bulk2 = pl.cdiv(
        (steps - split) * per_step - (_WRITE2_AT - _READ2_AT) * _FETCHES, per_step)
    assert bulk1 >= 1 and bulk2 >= 1
    for start, first, last, end in ((0, bulk1, split, _WRITE1_AT),
                                    (_READ2_AT, split + bulk2, steps, _WRITE2_AT)):
        assert _slot_free_at((first - 1) // 2) <= start
        for n in range(first * per_step, last * per_step):
            at = start + (n - first * per_step) // _FETCHES
            assert _slot_free_at(n // (2 * per_step)) <= at < min(end, n // per_step)
    assert _IN_SLOTS < _READ1_PIECES < pieces
    assert _slot_free_at(_READ1_PIECES - 1) < _WRITE1_AT < _READ2_AT < split
    assert _READ2_AT < _slot_free_at(pieces - 1) < _WRITE2_AT <= steps - 2

    written_at = {g: _WRITE1_AT for g in range(_AHEAD)}
    written_at.update({_WRITE1_GROUPS + g: _WRITE2_AT for g in range(_AHEAD)})
    for i in range(0, steps, 2):
        if i > _WRITE2_AT:
            written_at[_WRITE1_GROUPS + _AHEAD - 1 + i // 2 - _WRITE2_AT // 2] = i
        elif i > _WRITE1_AT and _AHEAD - 1 + i // 2 - _WRITE1_AT // 2 < _WRITE1_GROUPS:
            written_at[_AHEAD - 1 + i // 2 - _WRITE1_AT // 2] = i
    in_loop = len(written_at)
    assert sorted(written_at) == list(range(in_loop))
    assert groups - _OUT_SLOTS <= in_loop < groups
    assert all(4 * (g + 1) <= at < 4 * (g + _OUT_SLOTS) for g, at in written_at.items())
    assert written_at[_WRITE1_GROUPS - 1] < _READ2_AT
    assert _READ2_AT < 4 * (_WRITE1_GROUPS - 1 + _OUT_SLOTS) < steps
    return bulk1, bulk2, in_loop


@jax.jit
def pallas_standalone__detection_seg_fpn_lateral__vision_kernel(
    c_fine: jax.Array,
    p_coarse: jax.Array,
    w_lat: jax.Array,
    w_out: jax.Array,
):
    B, H, W, C = c_fine.shape
    Wc = W // 2
    units = B * H // 2
    bf16, f32 = jnp.bfloat16, jnp.float32
    assert c_fine.dtype == bf16 and units % _GROUP == 0

    steps, pieces, groups = units // _STEP, units // _PIECE, units // _GROUP
    bulk1, bulk2, groups_in_loop = _plan(steps, pieces, groups)
    last_pieces = (_READ1_PIECES - 1, pieces - 1)
    split = 2 * _READ1_PIECES
    per_step = _PARTS * _STEP
    part_rows = Wc // _PARTS
    dot_rows = 2 * W // _DOTS
    fine, coarse = pl.ds(0, 2 * W), pl.ds(2 * W, Wc)

    def kernel(c_hbm, p_hbm, wl_hbm, wo_hbm, o_hbm,
               in_buf, out_buf, wl_buf, wo_buf, wf_buf,
               c_sem, head_sem, p_sem, o_sem, w_sem):

        def piece_copy(k):
            slot = _rem(k, _IN_SLOTS)
            return pltpu.make_async_copy(
                c_hbm.at[pl.ds(k * _PIECE, _PIECE)],
                in_buf.at[pl.ds(slot * _PIECE, _PIECE), fine],
                c_sem.at[slot])

        def head_copies(k):
            u, slot = k * _PIECE, _rem(k, _IN_SLOTS) * _PIECE
            head = pl.ds(0, 2 * W - _TAIL)
            return (
                pltpu.make_async_copy(
                    c_hbm.at[pl.ds(u, _PIECE - 1)],
                    in_buf.at[pl.ds(slot, _PIECE - 1), fine], head_sem),
                pltpu.make_async_copy(
                    c_hbm.at[u + _PIECE - 1, head],
                    in_buf.at[slot + _PIECE - 1, head], head_sem),
            )

        def tail_copy(k):
            slot = _rem(k, _IN_SLOTS)
            tail = pl.ds(2 * W - _TAIL, _TAIL)
            return pltpu.make_async_copy(
                c_hbm.at[k * _PIECE + _PIECE - 1, tail],
                in_buf.at[slot * _PIECE + _PIECE - 1, tail], c_sem.at[slot])

        def coarse_step_copy(i):
            slot = _rem(i, 2 * _IN_SLOTS)
            return pltpu.make_async_copy(
                p_hbm.at[pl.ds(i * _STEP, _STEP)],
                in_buf.at[pl.ds(slot * _STEP, _STEP), coarse],
                p_sem.at[slot])

        def coarse_part_copy(n):
            u = lax.div(n, _PARTS)
            slot = lax.rem(u, _IN_SLOTS * _PIECE)
            row = pl.multiple_of(lax.rem(n, _PARTS) * part_rows, part_rows)
            return pltpu.make_async_copy(
                p_hbm.at[u, pl.ds(row, part_rows)],
                in_buf.at[slot, pl.ds(2 * W + row, part_rows)],
                p_sem.at[lax.div(slot, _STEP)])

        def write_start(g):
            slot = _rem(g, _OUT_SLOTS)
            for start in range(0, 2 * W, _RUN):
                cols = pl.ds(start, _RUN)
                pltpu.make_async_copy(
                    out_buf.at[pl.ds(slot * _GROUP, _GROUP), cols],
                    o_hbm.at[pl.ds(g * _GROUP, _GROUP), cols],
                    o_sem.at[slot]).start(priority=1)

        def write_wait(g):
            slot = _rem(g, _OUT_SLOTS)
            pltpu.make_async_copy(
                out_buf.at[pl.ds(slot * _GROUP, _GROUP)],
                o_hbm.at[pl.ds(g * _GROUP, _GROUP)],
                o_sem.at[slot]).wait()

        weights = (
            pltpu.make_async_copy(wl_hbm, wl_buf, w_sem.at[0]),
            pltpu.make_async_copy(wo_hbm, wo_buf, w_sem.at[1]),
        )
        for copy in weights:
            copy.start()
        piece_copy(0).start(priority=1)

        @pl.loop(0, bulk1)
        def _(i):
            coarse_step_copy(i).start(priority=1)

        @pl.loop(1, _IN_SLOTS)
        def _(k):
            piece_copy(k).start(priority=1)

        for copy in weights:
            copy.wait()
        wf_buf[...] = jnp.dot(
            wl_buf[...], wo_buf[...], preferred_element_type=f32).astype(bf16)

        @pl.loop(0, steps)
        def _(i):
            @pl.when((i == _WRITE1_AT) | (i == _WRITE2_AT))
            def _():
                first = i == _WRITE1_AT
                for copy in head_copies(jnp.where(first, *last_pieces)):
                    copy.wait()
                g0 = jnp.where(first, 0, _WRITE1_GROUPS)

                @pl.loop(0, _AHEAD)
                def _(n):
                    write_start(g0 + n)

            @pl.when(i == _READ2_AT)
            def _():
                write_wait(_WRITE1_GROUPS - 1)

                @pl.loop(split, split + bulk2)
                def _(n):
                    coarse_step_copy(n).start(priority=1)

                @pl.loop(_READ1_PIECES, _READ2_AT // 2 + _IN_SLOTS)
                def _(k):
                    piece_copy(k).start(priority=1)

            @pl.when((i & 1) == 0)
            def _():
                k = i >> 1
                nxt = k + (_IN_SLOTS - 1)

                @pl.when(((i > 0) & (nxt < last_pieces[0]))
                         | ((i > _READ2_AT) & (nxt < last_pieces[1])))
                def _():
                    piece_copy(nxt).start(priority=1)

                for last in last_pieces:
                    @pl.when(nxt == last)
                    def _():
                        for copy in head_copies(last):
                            copy.start(priority=1)
                        tail_copy(last).start(priority=1)

                g = k + jnp.where(
                    i > _WRITE2_AT,
                    _WRITE1_GROUPS + _AHEAD - 1 - _WRITE2_AT // 2,
                    _AHEAD - 1 - _WRITE1_AT // 2)

                @pl.when((i > _WRITE2_AT) | ((i > _WRITE1_AT) & (g < _WRITE1_GROUPS)))
                def _():
                    write_start(g)

                @pl.when((k != last_pieces[0]) & (k != last_pieces[1]))
                def _():
                    piece_copy(k).wait()

                for last in last_pieces:
                    @pl.when(k == last)
                    def _():
                        tail_copy(last).wait()

                old = (i >> 2) - _OUT_SLOTS

                @pl.when(((i & 3) == 0) & (old >= 0) & (old != _WRITE1_GROUPS - 1))
                def _():
                    write_wait(old)

            coarse_step_copy(i).wait()

            second = i >= _READ2_AT
            n0 = i * _FETCHES + jnp.where(
                second,
                (split + bulk2) * per_step - _READ2_AT * _FETCHES,
                bulk1 * per_step)
            n_end = jnp.where(second, steps * per_step, split * per_step)
            fetched = []

            def load(u, start, size):
                n = n0 + len(fetched)
                fetched.append(n)

                @pl.when(n < n_end)
                def _():
                    coarse_part_copy(n).start()

                return in_buf[u, pl.ds(start, size), :]

            u_in = lax.rem(i, 2 * _IN_SLOTS) * _STEP
            u_out = lax.rem(i, 4 * _OUT_SLOTS) * _STEP
            half = dot_rows // 2
            for r in range(_STEP):
                q = jnp.dot(load(u_in + r, 2 * W, Wc), wo_buf[...],
                            preferred_element_type=f32)
                q = jnp.concatenate([q, q], axis=0)
                for t in range(_DOTS):
                    start = t * dot_rows
                    if t == 0:
                        x = load(u_in + r, start, dot_rows)
                    else:
                        x = jnp.concatenate(
                            [load(u_in + r, start, half),
                             load(u_in + r, start + half, half)], axis=0)
                    x = pltpu.bitcast(x, jnp.uint32)
                    even = lax.bitcast_convert_type(x << 16, f32)
                    odd = lax.bitcast_convert_type(x & jnp.uint32(0xFFFF0000), f32)
                    y = jnp.dot(
                        jnp.concatenate([even, odd], axis=0).astype(bf16),
                        wf_buf[...], preferred_element_type=f32)
                    up = q[t * half:(t + 1) * half]
                    even, odd = (
                        lax.bitcast_convert_type(
                            (v + up).astype(bf16).astype(f32), jnp.uint32)
                        for v in (y[:half], y[half:]))
                    out_buf[u_out + r, pl.ds(start, dot_rows), :] = pltpu.bitcast(
                        (even >> 16) | odd, bf16)
            assert len(fetched) == _FETCHES

        @pl.loop(groups_in_loop, groups)
        def _(g):
            write_start(g)

        @pl.loop(groups - _OUT_SLOTS, groups)
        def _(g):
            write_wait(g)

    out = pl.pallas_call(
        kernel,
        in_specs=[pl.BlockSpec(memory_space=pl.ANY)] * 4,
        out_specs=pl.BlockSpec(memory_space=pl.ANY),
        out_shape=jax.ShapeDtypeStruct((units, 2 * W, C), bf16),
        scratch_shapes=[
            pltpu.VMEM((_IN_SLOTS * _PIECE, 2 * W + Wc, C), bf16),
            pltpu.VMEM((_OUT_SLOTS * _GROUP, 2 * W, C), bf16),
            pltpu.VMEM((C, C), bf16),
            pltpu.VMEM((C, C), bf16),
            pltpu.VMEM((C, C), bf16),
            pltpu.SemaphoreType.DMA((_IN_SLOTS,)),
            pltpu.SemaphoreType.DMA(()),
            pltpu.SemaphoreType.DMA((2 * _IN_SLOTS,)),
            pltpu.SemaphoreType.DMA((_OUT_SLOTS,)),
            pltpu.SemaphoreType.DMA((2,)),
        ],
        compiler_params=pltpu.CompilerParams(
            vmem_limit_bytes=110 * 1024 * 1024, disable_bounds_checks=True),
    )(
        c_fine.reshape(units, 2 * W, C),
        p_coarse.reshape(units, Wc, C),
        w_lat,
        w_out.reshape(C, C),
    )
    return out.reshape(B, H, W, C)
```
